```python
import os as _os
_os.environ.setdefault("JAX_PLATFORMS", "cpu")
import jax
import jax.numpy as jnp

def _softmax(x, axis=-1):
    return jax.nn.softmax(x, axis=axis)
def _gelu(x):
    return jax.nn.gelu(x, approximate=True)
def _silu(x):
    return jax.nn.silu(x)
def _sigmoid(x):
    return jax.nn.sigmoid(x)
def _layernorm(x, axis=-1, eps=1e-5):
    m = jnp.mean(x, axis=axis, keepdims=True)
    v = jnp.var(x, axis=axis, keepdims=True)
    return (x - m) / jnp.sqrt(v + eps)
def _scatter_add(tgt, idx, src, axis=0):
    return tgt.at[idx].add(src)
def _segment_sum(src, seg, n):
    return jax.ops.segment_sum(src, seg, n)
class _Rng:
    def __init__(self, key):
        self._k = key
    def _next(self):
        self._k, sub = jax.random.split(self._k)
        return sub
    def normal(self, shape):
        return jax.random.normal(self._next(), shape, dtype=jnp.bfloat16)
    def randint(self, lo, hi, shape):
        return jax.random.randint(self._next(), shape, lo, hi, dtype=jnp.int32)
    def uniform(self, shape, lo=0.0, hi=1.0):
        return jax.random.uniform(self._next(), shape, jnp.bfloat16, lo, hi)
    def permutation(self, n):
        return jax.random.permutation(self._next(), n)


kernel_name = 'concat_heads__gqa_block_cached__gqa_block_cached__near_ridge'

def setup_inputs():
    _rng = _Rng(jax.random.key(int.from_bytes(__import__("os").urandom(4), "little")))
    _w = (lambda a: (lambda t: t.astype(jnp.bfloat16) if jnp.issubdtype(t.dtype, jnp.floating) else t)(jnp.asarray(a)))
    def _A_setup():
        B, Sq, D = 16, 144, 448
        Hq, Hkv, Sk, Dh = 16, 8, 1024, 256
        assert Hq % Hkv == 0, (Hq, Hkv)
        return {
            "x": _w((lambda *s: _rng.normal(s) * 0.8)(B, Sq, D)),
            "k_cache": _w((lambda *s: _rng.normal(s) * 0.8)(B, Hkv, Sk, Dh)),
            "v_cache": _w((lambda *s: _rng.normal(s) * 0.05)(B, Hkv, Sk, Dh)),
            "wq": _w((lambda *s: _rng.normal(s) * 0.8)(D, Hq * Dh) * (D ** -0.5)),
            "wo": _w((lambda *s: _rng.normal(s) * 0.05)(Hq * Dh, D) * ((Hq * Dh) ** -0.5)),
        }
    _A_in = _A_setup()

    def _B_setup():
        B, Sq, D = 16, 144, 448
        Hq, Hkv, Sk, Dh = 16, 8, 1024, 256
        assert Hq % Hkv == 0, (Hq, Hkv)
        return {
            "x": _w((lambda *s: _rng.normal(s) * 0.8)(B, Sq, D)),
            "k_cache": _w((lambda *s: _rng.normal(s) * 0.8)(B, Hkv, Sk, Dh)),
            "v_cache": _w((lambda *s: _rng.normal(s) * 0.05)(B, Hkv, Sk, Dh)),
            "wq": _w((lambda *s: _rng.normal(s) * 0.8)(D, Hq * Dh) * (D ** -0.5)),
            "wo": _w((lambda *s: _rng.normal(s) * 0.05)(Hq * Dh, D) * ((Hq * Dh) ** -0.5)),
        }
    _B_in = _B_setup()

    return {
        "A_x": _A_in["x"],
        "A_k_cache": _A_in["k_cache"],
        "A_v_cache": _A_in["v_cache"],
        "A_wq": _A_in["wq"],
        "A_wo": _A_in["wo"],
        "B_x": _B_in["x"],
        "B_k_cache": _B_in["k_cache"],
        "B_v_cache": _B_in["v_cache"],
        "B_wq": _B_in["wq"],
        "B_wo": _B_in["wo"],
    }

def reference(A_x, A_k_cache, A_v_cache, A_wq, A_wo, B_x, B_k_cache, B_v_cache, B_wq, B_wo):
    def _A_ref(x, k_cache, v_cache, wq, wo):
        B, Sq, D = x.shape
        Hq, Dh = 16, 256
        Hkv = k_cache.shape[1]
        rep = Hq // Hkv
        q = (lambda x, *d: x.transpose(*d))((x @ wq).reshape(B, Sq, Hq, Dh), 0, 2, 1, 3)
        k = jnp.repeat(k_cache, rep, axis=1)
        v = jnp.repeat(v_cache, rep, axis=1)
        scores = jnp.einsum("bhqd,bhkd->bhqk", q, k) * (Dh ** -0.5)
        p = _softmax(scores, axis=-1)
        o = jnp.einsum("bhqk,bhkd->bhqd", p, v)
        return (lambda x, *d: x.transpose(*d))(o, 0, 2, 1, 3).reshape(B, Sq, Hq * Dh) @ wo

    def _B_ref(x, k_cache, v_cache, wq, wo):
        B, Sq, D = x.shape
        Hq, Dh = 16, 256
        Hkv = k_cache.shape[1]
        rep = Hq // Hkv
        q = (lambda x, *d: x.transpose(*d))((x @ wq).reshape(B, Sq, Hq, Dh), 0, 2, 1, 3)
        k = jnp.repeat(k_cache, rep, axis=1)
        v = jnp.repeat(v_cache, rep, axis=1)
        scores = jnp.einsum("bhqd,bhkd->bhqk", q, k) * (Dh ** -0.5)
        p = _softmax(scores, axis=-1)
        o = jnp.einsum("bhqk,bhkd->bhqd", p, v)
        return (lambda x, *d: x.transpose(*d))(o, 0, 2, 1, 3).reshape(B, Sq, Hq * Dh) @ wo

    a = _A_ref(A_x, A_k_cache, A_v_cache, A_wq, A_wo)
    b = _B_ref(B_x, B_k_cache, B_v_cache, B_wq, B_wo)
    return jnp.concatenate([a, b], axis=-1)
```

```python
import functools

import jax
import jax.numpy as jnp
from jax import lax
import jax.experimental.pallas as pl
import jax.experimental.pallas.tpu as pltpu

_HQ = 16
_DH = 256


def _kernel(xa_ref, ka_ref, va_ref, wqa_ref, woa_ref,
            xb_ref, kb_ref, vb_ref, wqb_ref, wob_ref,
            o_ref, acca_ref, accb_ref, *, rep, sq, d, n_h):
    h = pl.program_id(0)
    b = pl.program_id(1)
    scale = _DH ** -0.5

    def branch(x_ref, k_ref, v_ref, wq_ref, wo_ref):
        x = x_ref[0]
        q = jnp.dot(x, wq_ref[...], preferred_element_type=jnp.float32)
        q = (q * scale).astype(jnp.bfloat16)
        q2 = jnp.concatenate([q[:, r * _DH:(r + 1) * _DH] for r in range(rep)], axis=0)
        s = lax.dot_general(q2, k_ref[0, 0], (((1,), (1,)), ((), ())),
                            preferred_element_type=jnp.float32)
        m = jnp.max(s, axis=-1, keepdims=True)
        p = jnp.exp(s - m)
        l = jnp.sum(p, axis=-1, keepdims=True)
        o = jnp.dot(p.astype(jnp.bfloat16), v_ref[0, 0],
                    preferred_element_type=jnp.float32)
        o = (o / l).astype(jnp.bfloat16)
        oc = jnp.concatenate([o[r * sq:(r + 1) * sq] for r in range(rep)], axis=1)
        return jnp.dot(oc, wo_ref[...], preferred_element_type=jnp.float32)

    ya = branch(xa_ref, ka_ref, va_ref, wqa_ref, woa_ref)
    yb = branch(xb_ref, kb_ref, vb_ref, wqb_ref, wob_ref)

    @pl.when(h == 0)
    def _():
        acca_ref[b] = ya
        accb_ref[b] = yb

    @pl.when(jnp.logical_and(h > 0, h < n_h - 1))
    def _():
        acca_ref[b] += ya
        accb_ref[b] += yb

    @pl.when(h == n_h - 1)
    def _():
        o_ref[0, :, 0:d] = (acca_ref[b] + ya).astype(o_ref.dtype)
        o_ref[0, :, d:2 * d] = (accb_ref[b] + yb).astype(o_ref.dtype)


@jax.jit
def pallas_concat_heads__gqa_block_cached__gqa_block_cached__near_ridge_kernel(
    A_x: jax.Array,
    A_k_cache: jax.Array,
    A_v_cache: jax.Array,
    A_wq: jax.Array,
    A_wo: jax.Array,
    B_x: jax.Array,
    B_k_cache: jax.Array,
    B_v_cache: jax.Array,
    B_wq: jax.Array,
    B_wo: jax.Array,
):
    bsz, sq, d = A_x.shape
    _, hkv, sk, dh = A_k_cache.shape
    assert dh == _DH
    rep = _HQ // hkv
    gw = rep * dh

    x_spec = pl.BlockSpec((1, sq, d), lambda h, b: (b, 0, 0))
    kv_spec = pl.BlockSpec((1, 1, sk, dh), lambda h, b: (b, h, 0, 0))
    wq_spec = pl.BlockSpec((d, gw), lambda h, b: (0, h))
    wo_spec = pl.BlockSpec((gw, d), lambda h, b: (h, 0))
    out_spec = pl.BlockSpec(
        (1, sq, 2 * d), lambda h, b: (jnp.where(h == hkv - 1, b, 0), 0, 0))

    return pl.pallas_call(
        functools.partial(_kernel, rep=rep, sq=sq, d=d, n_h=hkv),
        grid=(hkv, bsz),
        in_specs=[x_spec, kv_spec, kv_spec, wq_spec, wo_spec] * 2,
        out_specs=out_spec,
        out_shape=jax.ShapeDtypeStruct((bsz, sq, 2 * d), A_x.dtype),
        scratch_shapes=[pltpu.VMEM((bsz, sq, d), jnp.float32),
                        pltpu.VMEM((bsz, sq, d), jnp.float32)],
        compiler_params=pltpu.CompilerParams(
            dimension_semantics=("arbitrary", "arbitrary"),
            vmem_limit_bytes=64 * 1024 * 1024),
    )(A_x, A_k_cache, A_v_cache, A_wq, A_wo, B_x, B_k_cache, B_v_cache, B_wq, B_wo)
```

```python
import functools
import math

import jax
import jax.numpy as jnp
from jax import lax
import jax.experimental.pallas as pl
import jax.experimental.pallas.tpu as pltpu

_HQ = 16
_DH = 256
_NB = 8
_NFINE = 2
_NT = (((1,), (1,)), ((), ()))
_RC = 16
_LANE = 128

_GROUPS = (((0, 0, 2), (1, 0, 1)), ((0, 2, 4), (1, 1, 3)),
           ((0, 4, 7), (1, 3, 6)), ((0, 7, 8), (1, 6, 8)))
_BARS = (('qk', 0), ('qk', 2), ('qk', 4), ('qk', 7))
_WO_BAR = 1
_ISSUE = {
    -1: (('x', 0), ('wq', 0)),
    0: (('kv', 0, 0), ('kv', 0, 1), ('wo', 0)),
    1: (('kv', 0, 2),),
    2: (('kv', 0, 3), ('x', 1)),
    3: (('kv', 1, 0), ('kv', 1, 1)),
    4: (('kv', 1, 2), ('kv', 1, 3)),
}


def _stage_order(nb):
    ops = []
    for t in range(nb + 2):
        if t < nb:
            ops.append(('qk', t))
        if 0 <= t - 2 and t < nb:
            ops.append(('o', t - 2))
        if 0 <= t - 1 < nb:
            ops.append(('pv', t - 1))
        if t >= nb:
            ops.append(('o', t - 2))
    return ops


def _zero_from(tok):
    t = pltpu.bitcast(tok, jnp.uint32)
    t = lax.shift_right_logical(lax.shift_right_logical(t, jnp.uint32(31)), jnp.uint32(1))
    return pltpu.bitcast(t, jnp.float32)


def _kernel(xa_hbm, ka_hbm, va_hbm, wqa_hbm, woa_hbm,
            xb_hbm, kb_hbm, vb_hbm, wqb_hbm, wob_hbm,
            o_hbm, acc_ref, x_buf, kv_buf, w_buf, o_buf, x_sem, kv_sem, w_sem, o_sem,
            *, rep, sq, d, n_h, nb, ng):
    step = pl.program_id(0)
    n_steps = n_h * 2 * ng
    last = n_steps - 1

    def coords(st):
        return st >> 2, (st >> 1) & 1, st & 1

    h, c, g = coords(step)
    scale = _DH ** -0.5 * math.log2(math.e)
    f32, bf16 = jnp.float32, jnp.bfloat16
    mr = rep * sq
    gw = rep * _DH
    n_t = nb * sq // _LANE
    n_grp = len(_GROUPS)

    x_hbm = (xa_hbm, xb_hbm)
    kv_hbm = ((ka_hbm, va_hbm), (kb_hbm, vb_hbm))
    w_hbm = ((wqa_hbm, woa_hbm), (wqb_hbm, wob_hbm))

    def x_copy(cs, cc, gg):
        return pltpu.make_async_copy(
            x_hbm[cs].at[pl.ds(gg * nb, nb)], x_buf.at[cc, gg], x_sem.at[cc * ng + gg])

    def w_copy(cs, j, hh, ws):
        col = hh * gw if isinstance(hh, int) else pl.multiple_of(hh * gw, gw)
        return pltpu.make_async_copy(
            w_hbm[cs][j].at[:, pl.ds(col, gw)], w_buf.at[ws, j], w_sem.at[ws * 2 + j])

    def kv_copy(cs, hh, gg, piece, gi):
        j, i0, i1 = piece
        return pltpu.make_async_copy(
            kv_hbm[cs][j].at[pl.ds(gg * nb + i0, i1 - i0), hh],
            kv_buf.at[gg, j, pl.ds(i0, i1 - i0)],
            kv_sem.at[gg * n_grp + gi])

    def kv_pieces(gi):
        return (((0, 0, nb), (1, 0, nb)), 0) if gi is None else (_GROUPS[gi], gi)

    def o_copy(gg, t):
        r0 = gg * (nb * sq) + t * _LANE
        return pltpu.make_async_copy(
            o_buf.at[gg, pl.ds(t * _LANE, _LANE)], o_hbm.at[pl.ds(r0, _LANE)], o_sem.at[gg])

    def issue(k):
        @pl.when(step == 0)
        def _():
            for pc in _ISSUE[k]:
                hh, cc, gg = coords(pc[1])
                if pc[0] == 'kv':
                    for piece in _GROUPS[pc[2]]:
                        kv_copy(cc, hh, gg, piece, pc[2]).start()
                elif pc[0] == 'x':
                    x_copy(cc, cc, gg).start()
                else:
                    w_copy(cc, 0 if pc[0] == 'wq' else 1, hh, cc).start()

    def prefetch(which):
        nstep = step + 1
        nh, nc, ngi = coords(nstep)
        pf_ok = jnp.logical_and(nstep >= _NFINE, nstep < n_steps)
        nh = jnp.minimum(nh, n_h - 1)
        for cs in range(2):
            ok = jnp.logical_and(pf_ok, nc == cs)
            if which == 'kv':
                for piece in kv_pieces(None)[0]:
                    @pl.when(ok)
                    def _():
                        kv_copy(cs, nh, ngi, piece, 0).start()
            else:
                if cs == 1:
                    @pl.when(jnp.logical_and(ok, nh == 0))
                    def _():
                        x_copy(cs, cs, ngi).start()
                for j in range(2):
                    @pl.when(jnp.logical_and(ok, ngi == 0))
                    def _():
                        w_copy(cs, j, nh, cs).start()

    def wait_x():
        @pl.when(h == 0)
        def _():
            x_copy(0, c, g).wait()

    def wait_w(j):
        @pl.when(g == 0)
        def _():
            w_copy(0, j, h, c).wait()

    def wait_kv(gi):
        pieces, si = kv_pieces(gi)
        for piece in pieces:
            kv_copy(0, h, g, piece, si).wait()

    def softmax(s, toks):
        ps, ls = [], []
        sk = s.shape[1]
        for j, r0 in enumerate(range(0, mr, _RC)):
            sc = s[r0:r0 + _RC]
            pm = sc[:, 0:_LANE]
            for cc in range(_LANE, sk, _LANE):
                pm = jnp.maximum(pm, sc[:, cc:cc + _LANE])
            z = _zero_from(toks[j])
            pm = pm + jnp.concatenate([z] * (_RC // 8), axis=0)
            m = jnp.max(pm, axis=-1, keepdims=True)
            e = jnp.exp2(sc - m)
            psum = e[:, 0:_LANE]
            for cc in range(_LANE, sk, _LANE):
                psum = psum + e[:, cc:cc + _LANE]
            ls.append(psum)
            ps.append(e.astype(bf16))
        return jnp.concatenate(ps, axis=0), jnp.concatenate(ls, axis=0)

    def toks_from(y, rounds, n):
        rows, cols = y.shape
        nrb = rows // 16
        cw = cols // rounds
        out = []
        for j in range(n):
            sl = (j * rounds * nrb) // n
            rd, rb = sl // nrb, sl % nrb
            out.append(y[rb * 16:rb * 16 + 8, rd * cw:rd * cw + _LANE])
        return out

    def body(special):
        s, oc, ys = {}, {}, {}
        n_tok = mr // _RC
        if special:
            issue(-1)
        wait_x()
        wait_w(0)
        if special:
            issue(0)

            @pl.when(step >= _NFINE)
            def _():
                wait_kv(None)
        else:
            wait_w(1)
            wait_kv(None)
        prefetch('kv')
        q = jnp.dot(x_buf[c, g].reshape(nb * sq, d), w_buf[c, 0], preferred_element_type=f32)
        q = (q * scale).astype(bf16)
        prefetch('w')

        def out_tile(gg, t):
            yt = acc_ref[gg, t].reshape(2 * d, _LANE)
            o_buf[gg, t * _LANE:(t + 1) * _LANE, :] = yt.T.astype(o_buf.dtype)

            @pl.when(step == last)
            def _():
                o_copy(gg, t).start()

        def do_qk(n):
            qn = q[n * sq:(n + 1) * sq]
            q2 = jnp.concatenate(
                [qn[:, r * _DH:(r + 1) * _DH] for r in range(rep)], axis=0)
            s[n] = lax.dot_general(q2, kv_buf[g, 0, n], _NT, preferred_element_type=f32)
            if special:
                out_tile(0, n)
                if n == nb - 1:
                    out_tile(0, nb)

        def do_pv(n):
            if n + 1 < nb:
                toks = toks_from(s[n + 1], 4, n_tok)
            else:
                toks = toks_from(ys[n - 2], 1, n_tok)
            p, psum = softmax(s[n], toks)
            o32 = jnp.dot(p, kv_buf[g, 1, n], preferred_element_type=f32)
            l = jnp.sum(psum + _zero_from(o32[:, 0:_LANE]), axis=-1, keepdims=True)
            o = (o32 * (1.0 / l)).astype(bf16)
            oc[n] = jnp.concatenate([o[r * sq:(r + 1) * sq] for r in range(rep)], axis=1)

        def do_o(n):
            wo = w_buf[c, 1]
            for t in range((n * sq) // _LANE, ((n + 1) * sq) // _LANE):
                r0, r1 = t * _LANE, (t + 1) * _LANE
                parts = []
                for ii in range(r0 // sq, (r1 - 1) // sq + 1):
                    a, b = max(r0, ii * sq) - ii * sq, min(r1, (ii + 1) * sq) - ii * sq
                    parts.append(oc[ii][a:b])
                ot = jnp.concatenate(parts, axis=0) if len(parts) > 1 else parts[0]
                y = lax.dot_general(wo, ot, _NT, preferred_element_type=f32)
                ys[n] = y
                prev = jnp.where(h == 0, 0.0, acc_ref[g, t, c])
                acc_ref[g, t, c] = prev + y
                if special:
                    out_tile(1, t)

        for stage in _stage_order(nb):
            if special and stage in _BARS:
                k = _BARS.index(stage)

                @pl.when(step < _NFINE)
                def _():
                    wait_kv(k)
                if k == _WO_BAR:
                    wait_w(1)
                issue(k + 1)
            {'qk': do_qk, 'pv': do_pv, 'o': do_o}[stage[0]](stage[1])

        if special:
            @pl.when(step == last)
            def _():
                for gg in range(ng):
                    for t in range(n_t):
                        o_copy(gg, t).wait()

    is_special = jnp.logical_or(step < _NFINE, step == last)

    @pl.when(is_special)
    def _():
        body(True)

    @pl.when(jnp.logical_not(is_special))
    def _():
        body(False)


@jax.jit
def pallas_concat_heads__gqa_block_cached__gqa_block_cached__near_ridge_kernel(
    A_x: jax.Array,
    A_k_cache: jax.Array,
    A_v_cache: jax.Array,
    A_wq: jax.Array,
    A_wo: jax.Array,
    B_x: jax.Array,
    B_k_cache: jax.Array,
    B_v_cache: jax.Array,
    B_wq: jax.Array,
    B_wo: jax.Array,
):
    bsz, sq, d = A_x.shape
    _, hkv, sk, dh = A_k_cache.shape
    rep = _HQ // hkv
    gw = rep * dh
    nb = _NB
    ng = bsz // nb
    dt = A_x.dtype
    rows = nb * sq
    assert dh == _DH and ng == 2 and rows % _LANE == 0 and sq % 16 == 0
    n_steps = hkv * 2 * ng

    any_spec = pl.BlockSpec(memory_space=pl.ANY)
    out = pl.pallas_call(
        functools.partial(_kernel, rep=rep, sq=sq, d=d, n_h=hkv, nb=nb, ng=ng),
        grid=(n_steps,),
        in_specs=[any_spec] * 10,
        out_specs=any_spec,
        out_shape=jax.ShapeDtypeStruct((bsz * sq, 2 * d), dt),
        scratch_shapes=[pltpu.VMEM((ng, rows // _LANE, 2, d, _LANE), jnp.float32),
                        pltpu.VMEM((2, ng, nb, sq, d), dt),
                        pltpu.VMEM((ng, 2, nb, sk, dh), dt),
                        pltpu.VMEM((2, 2, d, gw), dt),
                        pltpu.VMEM((ng, rows, 2 * d), dt),
                        pltpu.SemaphoreType.DMA((2 * ng,)),
                        pltpu.SemaphoreType.DMA((ng * len(_GROUPS),)),
                        pltpu.SemaphoreType.DMA((4,)),
                        pltpu.SemaphoreType.DMA((ng,))],
        compiler_params=pltpu.CompilerParams(
            dimension_semantics=("arbitrary",),
            disable_bounds_checks=True,
            vmem_limit_bytes=100 * 1024 * 1024),
    )(A_x, A_k_cache, A_v_cache, A_wq, A_wo.T, B_x, B_k_cache, B_v_cache, B_wq, B_wo.T)
    return out.reshape(bsz, sq, 2 * d)
```

```python
import functools
import math

import jax
import jax.numpy as jnp
from jax import lax
import jax.experimental.pallas as pl
import jax.experimental.pallas.tpu as pltpu

_HQ = 16
_DH = 256
_NB = 8
_NFINE = 2
_NT = (((1,), (1,)), ((), ()))
_RC = 16
_LANE = 128

_GROUPS = (((0, 0, 2), (1, 0, 1)), ((0, 2, 4), (1, 1, 3)),
           ((0, 4, 7), (1, 3, 6)), ((0, 7, 8), (1, 6, 8)))
_BARS = (('qk', 0), ('qk', 2), ('qk', 4), ('qk', 7))
_WO_BAR = 1
_ISSUE = {
    -1: (('x', 0), ('wq', 0)),
    0: (('kv', 0, 0), ('kv', 0, 1), ('wo', 0)),
    1: (('kv', 0, 2),),
    2: (('kv', 0, 3),),
    3: (('x', 1), ('kv', 1, 0), ('kv', 1, 1)),
    4: (('kv', 1, 2), ('kv', 1, 3)),
}


def _stage_order(nb):
    ops = []
    for t in range(nb + 2):
        if t < nb:
            ops.append(('qk', t))
        if 2 <= t < nb:
            ops.append(('o', t - 2))
        if 1 <= t <= nb:
            ops.append(('pv', t - 1))
        if t >= nb:
            ops.append(('o', t - 2))
    return ops


def _zero_from(tok):
    t = pltpu.bitcast(tok, jnp.uint32)
    t = lax.shift_right_logical(lax.shift_right_logical(t, jnp.uint32(31)), jnp.uint32(1))
    return pltpu.bitcast(t, jnp.float32)


def _kernel(xa_hbm, ka_hbm, va_hbm, wqa_hbm, woa_hbm,
            xb_hbm, kb_hbm, vb_hbm, wqb_hbm, wob_hbm,
            o_hbm, acc_ref, x_buf, kv_buf, w_buf, o_buf, x_sem, kv_sem, w_sem, o_sem,
            *, rep, sq, d, n_h, nb, ng):
    n_steps = n_h * 2 * ng
    last = n_steps - 1

    def coords(st):
        return st >> 2, (st >> 1) & 1, st & 1

    scale = _DH ** -0.5 * math.log2(math.e)
    f32, bf16 = jnp.float32, jnp.bfloat16
    mr = rep * sq
    gw = rep * _DH
    n_t = nb * sq // _LANE
    n_grp = len(_GROUPS)
    c_mid = (d // _LANE) * _LANE

    x_hbm = (xa_hbm, xb_hbm)
    kv_hbm = ((ka_hbm, va_hbm), (kb_hbm, vb_hbm))
    w_hbm = ((wqa_hbm, woa_hbm), (wqb_hbm, wob_hbm))

    def x_copy(cs, gg):
        return pltpu.make_async_copy(
            x_hbm[cs].at[pl.ds(gg * nb, nb)], x_buf.at[cs, gg], x_sem.at[cs * ng + gg])

    def w_copy(cs, j, hh, ws):
        col = hh * gw if isinstance(hh, int) else pl.multiple_of(hh * gw, gw)
        return pltpu.make_async_copy(
            w_hbm[cs][j].at[:, pl.ds(col, gw)], w_buf.at[ws, j], w_sem.at[ws * 2 + j])

    def kv_copy(cs, hh, gg, piece, gi):
        j, i0, i1 = piece
        return pltpu.make_async_copy(
            kv_hbm[cs][j].at[pl.ds(gg * nb + i0, i1 - i0), hh],
            kv_buf.at[gg, j, pl.ds(i0, i1 - i0)],
            kv_sem.at[gg * n_grp + gi])

    def kv_pieces(gi):
        return (((0, 0, nb), (1, 0, nb)), 0) if gi is None else (_GROUPS[gi], gi)

    def o_copy(gg, t0, t1, c0, c1, si):
        r0 = gg * (nb * sq) + t0 * _LANE
        n_r = (t1 - t0) * _LANE
        return pltpu.make_async_copy(
            o_buf.at[gg, pl.ds(t0 * _LANE, n_r), pl.ds(c0, c1 - c0)],
            o_hbm.at[pl.ds(r0, n_r), pl.ds(c0, c1 - c0)], o_sem.at[si])

    def softmax(s, toks):
        ps, ls = [], []
        sk = s.shape[1]
        for j, r0 in enumerate(range(0, mr, _RC)):
            sc = s[r0:r0 + _RC]
            pm = sc[:, 0:_LANE]
            for cc in range(_LANE, sk, _LANE):
                pm = jnp.maximum(pm, sc[:, cc:cc + _LANE])
            z = _zero_from(toks[j])
            pm = pm + jnp.concatenate([z] * (_RC // 8), axis=0)
            m = jnp.max(pm, axis=-1, keepdims=True)
            e = jnp.exp2(sc - m)
            psum = e[:, 0:_LANE]
            for cc in range(_LANE, sk, _LANE):
                psum = psum + e[:, cc:cc + _LANE]
            ls.append(psum)
            ps.append(e.astype(bf16))
        return jnp.concatenate(ps, axis=0), jnp.concatenate(ls, axis=0)

    def toks_from(y, rounds, n):
        rows, cols = y.shape
        nrb = rows // 16
        cw = cols // rounds
        out = []
        for j in range(n):
            sl = (j * rounds * nrb) // n
            rd, rb = sl // nrb, sl % nrb
            out.append(y[rb * 16:rb * 16 + 8, rd * cw:rd * cw + _LANE])
        return out

    def body(step, special):
        h, c, g = coords(step)
        s, oc, ys = {}, {}, {}
        n_tok = mr // _RC

        def issue(k):
            @pl.when(step == 0)
            def _():
                for pc in _ISSUE[k]:
                    hh, cc, gg = coords(pc[1])
                    if pc[0] == 'kv':
                        for piece in _GROUPS[pc[2]]:
                            kv_copy(cc, hh, gg, piece, pc[2]).start()
                    elif pc[0] == 'x':
                        x_copy(cc, gg).start()
                    else:
                        w_copy(cc, 0 if pc[0] == 'wq' else 1, hh, cc).start()

        def prefetch(which):
            nh, nc, ngi = coords(step + 1)
            if special:
                nh = jnp.minimum(nh, n_h - 1)
            for cs in range(2):
                ok = nc == cs
                if special:
                    ok = jnp.logical_and(ok, step == _NFINE - 1)
                if which == 'kv':
                    for piece in kv_pieces(None)[0]:
                        @pl.when(ok)
                        def _():
                            kv_copy(cs, nh, ngi, piece, 0).start()
                else:
                    if cs == 1:
                        @pl.when(jnp.logical_and(ok, nh == 0))
                        def _():
                            x_copy(cs, ngi).start()
                    for j in range(2):
                        @pl.when(jnp.logical_and(ok, ngi == 0))
                        def _():
                            w_copy(cs, j, nh, cs).start()

        def wait_w(j):
            @pl.when(g == 0)
            def _():
                w_copy(0, j, h, c).wait()

        def wait_kv(gi):
            pieces, si = kv_pieces(gi)
            for piece in pieces:
                kv_copy(0, h, g, piece, si).wait()

        def out_start(gg, t0, t1, c0, c1, si):
            @pl.when(step == last)
            def _():
                o_copy(gg, t0, t1, c0, c1, si).start()

        if special:
            issue(-1)

            @pl.when(step < _NFINE)
            def _():
                x_copy(0, g).wait()
            wait_w(0)
            issue(0)

            @pl.when(step >= _NFINE)
            def _():
                wait_kv(None)
        else:
            @pl.when(h == 0)
            def _():
                x_copy(1, g).wait()
            wait_w(0)
            wait_w(1)
            wait_kv(None)
        prefetch('kv')
        q = jnp.dot(x_buf[c, g].reshape(nb * sq, d), w_buf[c, 0], preferred_element_type=f32)
        q = (q * scale).astype(bf16)
        prefetch('w')

        if special:
            for gg, c1, si in ((0, 2 * d, 0), (1, c_mid, 1)):
                for t in range(n_t):
                    yt = acc_ref[gg, t].reshape(2 * d, _LANE)[0:c1]
                    o_buf[gg, t * _LANE:(t + 1) * _LANE, 0:c1] = yt.T.astype(o_buf.dtype)
                out_start(gg, 0, n_t, 0, c1, si)

        def do_qk(n):
            qn = q[n * sq:(n + 1) * sq]
            q2 = jnp.concatenate(
                [qn[:, r * _DH:(r + 1) * _DH] for r in range(rep)], axis=0)
            s[n] = lax.dot_general(q2, kv_buf[g, 0, n], _NT, preferred_element_type=f32)

        def do_pv(n):
            if n + 1 < nb:
                toks = toks_from(s[n + 1], 4, n_tok)
            else:
                toks = toks_from(ys[n - 2], 1, n_tok)
            p, psum = softmax(s[n], toks)
            o32 = jnp.dot(p, kv_buf[g, 1, n], preferred_element_type=f32)
            l = jnp.sum(psum + _zero_from(o32[:, 0:_LANE]), axis=-1, keepdims=True)
            r0 = pl.reciprocal(l, approx=True)
            o = o32 * (r0 * (2.0 - l * r0))
            oc[n] = jnp.concatenate([o[r * sq:(r + 1) * sq] for r in range(rep)], axis=1)

        def do_o(n):
            wo = w_buf[c, 1]
            for t in range((n * sq) // _LANE, ((n + 1) * sq) // _LANE):
                r0, r1 = t * _LANE, (t + 1) * _LANE
                parts = []
                for ii in range(r0 // sq, (r1 - 1) // sq + 1):
                    a, b = max(r0, ii * sq) - ii * sq, min(r1, (ii + 1) * sq) - ii * sq
                    parts.append(oc[ii][a:b])
                ot = jnp.concatenate(parts, axis=0) if len(parts) > 1 else parts[0]
                if special:
                    a_tail = acc_ref[1, t, 0, c_mid:d, :]
                y = lax.dot_general(wo, ot.astype(bf16), _NT, preferred_element_type=f32)
                ys[n] = y
                new = jnp.where(h == 0, 0.0, acc_ref[g, t, c]) + y
                acc_ref[g, t, c] = new
                if special:
                    yt = jnp.concatenate([a_tail, new], axis=0)
                    o_buf[1, r0:r1, c_mid:2 * d] = yt.T.astype(o_buf.dtype)
                    out_start(1, t, t + 1, c_mid, 2 * d, 2)

        for stage in _stage_order(nb):
            if special and stage in _BARS:
                k = _BARS.index(stage)

                @pl.when(step < _NFINE)
                def _():
                    wait_kv(k)
                if k == _WO_BAR:
                    wait_w(1)
                issue(k + 1)
            {'qk': do_qk, 'pv': do_pv, 'o': do_o}[stage[0]](stage[1])

        if special:
            @pl.when(step == last)
            def _():
                o_copy(0, 0, n_t, 0, 2 * d, 0).wait()
                o_copy(1, 0, n_t, 0, c_mid, 1).wait()
                for t in range(n_t):
                    o_copy(1, t, t + 1, c_mid, 2 * d, 2).wait()

    i = pl.program_id(0)
    body(jnp.where(i < _NFINE, i, last), True)

    def loop_body(st, carry):
        body(st, False)
        return carry

    lax.fori_loop(_NFINE, jnp.where(i == _NFINE - 1, last, _NFINE), loop_body, 0)


@jax.jit
def pallas_concat_heads__gqa_block_cached__gqa_block_cached__near_ridge_kernel(
    A_x: jax.Array,
    A_k_cache: jax.Array,
    A_v_cache: jax.Array,
    A_wq: jax.Array,
    A_wo: jax.Array,
    B_x: jax.Array,
    B_k_cache: jax.Array,
    B_v_cache: jax.Array,
    B_wq: jax.Array,
    B_wo: jax.Array,
):
    bsz, sq, d = A_x.shape
    _, hkv, sk, dh = A_k_cache.shape
    rep = _HQ // hkv
    gw = rep * dh
    nb = _NB
    ng = bsz // nb
    dt = A_x.dtype
    rows = nb * sq
    assert dh == _DH and ng == 2 and rows % _LANE == 0 and sq % 16 == 0

    any_spec = pl.BlockSpec(memory_space=pl.ANY)
    out = pl.pallas_call(
        functools.partial(_kernel, rep=rep, sq=sq, d=d, n_h=hkv, nb=nb, ng=ng),
        grid=(_NFINE + 1,),
        in_specs=[any_spec] * 10,
        out_specs=any_spec,
        out_shape=jax.ShapeDtypeStruct((bsz * sq, 2 * d), dt),
        scratch_shapes=[pltpu.VMEM((ng, rows // _LANE, 2, d, _LANE), jnp.float32),
                        pltpu.VMEM((2, ng, nb, sq, d), dt),
                        pltpu.VMEM((ng, 2, nb, sk, dh), dt),
                        pltpu.VMEM((2, 2, d, gw), dt),
                        pltpu.VMEM((ng, rows, 2 * d), dt),
                        pltpu.SemaphoreType.DMA((2 * ng,)),
                        pltpu.SemaphoreType.DMA((ng * len(_GROUPS),)),
                        pltpu.SemaphoreType.DMA((4,)),
                        pltpu.SemaphoreType.DMA((3,))],
        compiler_params=pltpu.CompilerParams(
            dimension_semantics=("arbitrary",),
            disable_bounds_checks=True,
            vmem_limit_bytes=100 * 1024 * 1024),
    )(A_x, A_k_cache, A_v_cache, A_wq, A_wo.T, B_x, B_k_cache, B_v_cache, B_wq, B_wo.T)
    return out.reshape(bsz, sq, 2 * d)
```

```python
import functools
import math

import jax
import jax.numpy as jnp
from jax import lax
import jax.experimental.pallas as pl
import jax.experimental.pallas.tpu as pltpu

_HQ = 16
_DH = 256
_NB = 8
_NFINE = 2
_NT = (((1,), (1,)), ((), ()))
_RC = 16
_LANE = 128

_GROUPS = (((0, 0, 2), (1, 0, 1)), ((0, 2, 4), (1, 1, 3)),
           ((0, 4, 6), (1, 3, 5)), ((0, 6, 8), (1, 5, 8)))
_BARS = (('qk', 0), ('qk', 2), ('qk', 4), ('qk', 6))
_WO_BAR = 1
_ISSUE = {
    -1: (('x', 0), ('wq', 0)),
    0: (('kv', 0, 0), ('kv', 0, 1), ('wo', 0)),
    1: (('kv', 0, 2),),
    2: (('kv', 0, 3),),
    'p3': (('wq', 1),),
    3: (('kv', 1, 0), ('kv', 1, 1)),
    'p4': (('wo', 1),),
    4: (('kv', 1, 2), ('kv', 1, 3)),
}


def _stage_order(nb):
    ops = []
    for t in range(nb + 2):
        if t < nb:
            ops.append(('qk', t))
        if 2 <= t < nb:
            ops.append(('o', t - 2))
        if 1 <= t <= nb:
            ops.append(('pv', t - 1))
        if t >= nb:
            ops.append(('o', t - 2))
    return ops


def _zero_from(tok):
    t = pltpu.bitcast(tok, jnp.uint32)
    t = lax.shift_right_logical(lax.shift_right_logical(t, jnp.uint32(31)), jnp.uint32(1))
    return pltpu.bitcast(t, jnp.float32)


def _kernel(xa_hbm, ka_hbm, va_hbm, wqa_hbm, woa_hbm,
            xb_hbm, kb_hbm, vb_hbm, wqb_hbm, wob_hbm,
            o_hbm, acc_ref, x_buf, kv_buf, w_buf, o_buf, x_sem, kv_sem, w_sem, o_sem,
            *, rep, sq, d, n_h, nb, ng):
    n_steps = n_h * 2 * ng
    last = n_steps - 1
    hb = n_h.bit_length() - 1

    def coords(st):
        return st >> (hb + 1), (st >> hb) & 1, st & (n_h - 1), st & 1

    scale = _DH ** -0.5 * math.log2(math.e)
    f32, bf16 = jnp.float32, jnp.bfloat16
    mr = rep * sq
    gw = rep * _DH
    n_t = nb * sq // _LANE
    n_grp = len(_GROUPS)
    c_mid = (d // _LANE) * _LANE
    whole = ((0, 0, nb), (1, 0, nb))

    x_hbm = (xa_hbm, xb_hbm)
    kv_hbm = ((ka_hbm, va_hbm), (kb_hbm, vb_hbm))
    w_hbm = ((wqa_hbm, woa_hbm), (wqb_hbm, wob_hbm))

    def x_copy(cs, gg):
        return pltpu.make_async_copy(
            x_hbm[cs].at[pl.ds(gg * nb, nb)], x_buf.at[gg], x_sem.at[gg])

    def w_copy(cs, j, hh, sl, fine):
        col = hh * gw if isinstance(hh, int) else pl.multiple_of(hh * gw, gw)
        sem = w_sem.at[sl * 2 + j] if fine else kv_sem.at[sl * n_grp]
        return pltpu.make_async_copy(
            w_hbm[cs][j].at[:, pl.ds(col, gw)], w_buf.at[sl, j], sem)

    def kv_copy(cs, gg, hh, sl, piece, gi):
        j, i0, i1 = piece
        return pltpu.make_async_copy(
            kv_hbm[cs][j].at[pl.ds(gg * nb + i0, i1 - i0), hh],
            kv_buf.at[sl, j, pl.ds(i0, i1 - i0)],
            kv_sem.at[sl * n_grp + gi])

    def o_copy(gg, t0, t1, c0, c1, si):
        r0 = gg * (nb * sq) + t0 * _LANE
        n_r = (t1 - t0) * _LANE
        return pltpu.make_async_copy(
            o_buf.at[gg, pl.ds(t0 * _LANE, n_r), pl.ds(c0, c1 - c0)],
            o_hbm.at[pl.ds(r0, n_r), pl.ds(c0, c1 - c0)], o_sem.at[si])

    def softmax(s, toks):
        ps, ls = [], []
        sk = s.shape[1]
        for j, r0 in enumerate(range(0, mr, _RC)):
            sc = s[r0:r0 + _RC]
            pm = sc[:, 0:_LANE]
            for cc in range(_LANE, sk, _LANE):
                pm = jnp.maximum(pm, sc[:, cc:cc + _LANE])
            z = _zero_from(toks[j])
            pm = pm + jnp.concatenate([z] * (_RC // 8), axis=0)
            m = jnp.max(pm, axis=-1, keepdims=True)
            e = jnp.exp2(sc - m)
            psum = e[:, 0:_LANE]
            for cc in range(_LANE, sk, _LANE):
                psum = psum + e[:, cc:cc + _LANE]
            ls.append(psum)
            ps.append(e.astype(bf16))
        return jnp.concatenate(ps, axis=0), jnp.concatenate(ls, axis=0)

    def toks_from(y, rounds, n):
        rows, cols = y.shape
        nrb = rows // 16
        cw = cols // rounds
        out = []
        for j in range(n):
            sl = (j * rounds * nrb) // n
            rd, rb = sl // nrb, sl % nrb
            out.append(y[rb * 16:rb * 16 + 8, rd * cw:rd * cw + _LANE])
        return out

    def body(step, special):
        c, g, h, slot = coords(step)
        s, oc, ys = {}, {}, {}
        n_tok = mr // _RC

        def issue(k):
            if k not in _ISSUE:
                return

            @pl.when(step == 0)
            def _():
                for pc in _ISSUE[k]:
                    cc, gg, hh, sl = coords(pc[1])
                    if pc[0] == 'kv':
                        for piece in _GROUPS[pc[2]]:
                            kv_copy(cc, gg, hh, sl, piece, pc[2]).start()
                    elif pc[0] == 'x':
                        x_copy(cc, gg).start()
                    else:
                        w_copy(cc, 0 if pc[0] == 'wq' else 1, hh, sl, True).start()

        def prefetch(which):
            if special:
                nc, ngi, nh, nsl = coords(_NFINE)

                @pl.when(step == _NFINE - 1)
                def _():
                    for j in range(2):
                        w_copy(nc, j, nh, nsl, False).start()
                    for piece in whole:
                        kv_copy(nc, ngi, nh, nsl, piece, 0).start()
                return
            nc, ngi, nh, nsl = coords(step + 1)
            for cs in range(2):
                ok = nc == cs
                if which == 'kv':
                    for piece in whole:
                        @pl.when(ok)
                        def _():
                            kv_copy(cs, ngi, nh, nsl, piece, 0).start()
                else:
                    @pl.when(jnp.logical_and(ok, nh == 0))
                    def _():
                        x_copy(cs, ngi).start()
                    for j in range(2):
                        @pl.when(ok)
                        def _():
                            w_copy(cs, j, nh, nsl, False).start()

        def wait_all():
            for j in range(2):
                w_copy(0, j, h, slot, False).wait()
            for piece in whole:
                kv_copy(0, g, h, slot, piece, 0).wait()

        def out_start(gg, t0, t1, c0, c1, si):
            @pl.when(step == last)
            def _():
                o_copy(gg, t0, t1, c0, c1, si).start()

        if special:
            issue(-1)

            @pl.when(step == 0)
            def _():
                x_copy(0, 0).wait()

            @pl.when(step < _NFINE)
            def _():
                w_copy(0, 0, h, slot, True).wait()
            issue(0)
            prefetch('all')

            @pl.when(step >= _NFINE)
            def _():
                wait_all()
        else:
            @pl.when(h == 0)
            def _():
                x_copy(0, g).wait()
            wait_all()
            prefetch('kv')
        xx = x_buf[g].reshape(nb * sq, d)
        q = jnp.dot(xx[:, c_mid:], w_buf[slot, 0, c_mid:, :], preferred_element_type=f32)
        q = jnp.dot(xx[:, :c_mid], w_buf[slot, 0, :c_mid, :], preferred_element_type=f32) + q
        q = (q * scale).astype(bf16)
        if not special:
            prefetch('w')

        if special:
            for gg, c1, si in ((0, 2 * d, 0), (1, c_mid, 1)):
                for t in range(n_t):
                    yt = acc_ref[gg, t].reshape(2 * d, _LANE)[0:c1]
                    o_buf[gg, t * _LANE:(t + 1) * _LANE, 0:c1] = yt.T.astype(o_buf.dtype)
                out_start(gg, 0, n_t, 0, c1, si)

        def do_qk(n):
            qn = q[n * sq:(n + 1) * sq]
            q2 = jnp.concatenate(
                [qn[:, r * _DH:(r + 1) * _DH] for r in range(rep)], axis=0)
            s[n] = lax.dot_general(q2, kv_buf[slot, 0, n], _NT, preferred_element_type=f32)

        def do_pv(n):
            if n + 1 < nb:
                toks = toks_from(s[n + 1], 4, n_tok)
            else:
                toks = toks_from(ys[n - 2], 1, n_tok)
            p, psum = softmax(s[n], toks)
            o32 = jnp.dot(p, kv_buf[slot, 1, n], preferred_element_type=f32)
            l = jnp.sum(psum + _zero_from(o32[:, 0:_LANE]), axis=-1, keepdims=True)
            r0 = pl.reciprocal(l, approx=True)
            o = o32 * (r0 * (2.0 - l * r0))
            oc[n] = jnp.concatenate([o[r * sq:(r + 1) * sq] for r in range(rep)], axis=1)

        def do_o(n):
            wo = w_buf[slot, 1]
            for t in range((n * sq) // _LANE, ((n + 1) * sq) // _LANE):
                r0, r1 = t * _LANE, (t + 1) * _LANE
                parts = []
                for ii in range(r0 // sq, (r1 - 1) // sq + 1):
                    a, b = max(r0, ii * sq) - ii * sq, min(r1, (ii + 1) * sq) - ii * sq
                    parts.append(oc[ii][a:b])
                ot = jnp.concatenate(parts, axis=0) if len(parts) > 1 else parts[0]
                if special:
                    a_tail = acc_ref[1, t, 0, c_mid:d, :]
                y = lax.dot_general(wo, ot.astype(bf16), _NT, preferred_element_type=f32)
                ys[n] = y
                new = jnp.where(h == 0, 0.0, acc_ref[g, t, c]) + y
                acc_ref[g, t, c] = new
                if special:
                    yt = jnp.concatenate([a_tail, new], axis=0)
                    o_buf[1, r0:r1, c_mid:2 * d] = yt.T.astype(o_buf.dtype)
                    out_start(1, t, t + 1, c_mid, 2 * d, 2)

        for stage in _stage_order(nb):
            if special and stage in _BARS:
                k = _BARS.index(stage)
                issue('p%d' % (k + 1))

                @pl.when(step < _NFINE)
                def _():
                    for piece in _GROUPS[k]:
                        kv_copy(0, g, h, slot, piece, k).wait()
                    if k == _WO_BAR:
                        w_copy(0, 1, h, slot, True).wait()
                issue(k + 1)
            {'qk': do_qk, 'pv': do_pv, 'o': do_o}[stage[0]](stage[1])

        if special:
            @pl.when(step == last)
            def _():
                o_copy(0, 0, n_t, 0, 2 * d, 0).wait()
                o_copy(1, 0, n_t, 0, c_mid, 1).wait()
                for t in range(n_t):
                    o_copy(1, t, t + 1, c_mid, 2 * d, 2).wait()

    i = pl.program_id(0)
    body(jnp.where(i < _NFINE, i, last), True)

    def loop_body(st, carry):
        body(st, False)
        return carry

    lax.fori_loop(_NFINE, jnp.where(i == _NFINE - 1, last, _NFINE), loop_body, 0)


@jax.jit
def pallas_concat_heads__gqa_block_cached__gqa_block_cached__near_ridge_kernel(
    A_x: jax.Array,
    A_k_cache: jax.Array,
    A_v_cache: jax.Array,
    A_wq: jax.Array,
    A_wo: jax.Array,
    B_x: jax.Array,
    B_k_cache: jax.Array,
    B_v_cache: jax.Array,
    B_wq: jax.Array,
    B_wo: jax.Array,
):
    bsz, sq, d = A_x.shape
    _, hkv, sk, dh = A_k_cache.shape
    rep = _HQ // hkv
    gw = rep * dh
    nb = _NB
    ng = bsz // nb
    dt = A_x.dtype
    rows = nb * sq
    assert dh == _DH and ng == 2 and rows % _LANE == 0 and sq % 16 == 0
    assert hkv & (hkv - 1) == 0 and hkv > _NFINE

    any_spec = pl.BlockSpec(memory_space=pl.ANY)
    out = pl.pallas_call(
        functools.partial(_kernel, rep=rep, sq=sq, d=d, n_h=hkv, nb=nb, ng=ng),
        grid=(_NFINE + 1,),
        in_specs=[any_spec] * 10,
        out_specs=any_spec,
        out_shape=jax.ShapeDtypeStruct((bsz * sq, 2 * d), dt),
        scratch_shapes=[pltpu.VMEM((ng, rows // _LANE, 2, d, _LANE), jnp.float32),
                        pltpu.VMEM((ng, nb, sq, d), dt),
                        pltpu.VMEM((2, 2, nb, sk, dh), dt),
                        pltpu.VMEM((2, 2, d, gw), dt),
                        pltpu.VMEM((ng, rows, 2 * d), dt),
                        pltpu.SemaphoreType.DMA((ng,)),
                        pltpu.SemaphoreType.DMA((2 * len(_GROUPS),)),
                        pltpu.SemaphoreType.DMA((4,)),
                        pltpu.SemaphoreType.DMA((3,))],
        compiler_params=pltpu.CompilerParams(
            dimension_semantics=("arbitrary",),
            disable_bounds_checks=True,
            vmem_limit_bytes=100 * 1024 * 1024),
    )(A_x, A_k_cache, A_v_cache, A_wq, A_wo.T, B_x, B_k_cache, B_v_cache, B_wq, B_wo.T)
    return out.reshape(bsz, sq, 2 * d)
```

```python
import functools
import math

import jax
import jax.numpy as jnp
from jax import lax
import jax.experimental.pallas as pl
import jax.experimental.pallas.tpu as pltpu

_HQ = 16
_DH = 256
_NB = 8
_NFINE = 2
_NT = (((1,), (1,)), ((), ()))
_RC = 16
_LANE = 128

_GROUPS = (((0, 0, 2), (1, 0, 1)), ((0, 2, 4), (1, 1, 3)),
           ((0, 4, 6), (1, 3, 5)), ((0, 6, 8), (1, 5, 8)))
_BARS = (('qk', 0), ('qk', 2), ('qk', 4), ('qk', 6))
_WO_BAR = 1
_ISSUE = {
    -1: (('x', 0), ('wq', 0), ('kv', 0, 0), ('kv', 0, 1)),
    0: (('wo', 0),),
    1: (('kv', 0, 2),),
    2: (('kv', 0, 3),),
    'p3': (('wq', 1),),
    3: (('kv', 1, 0), ('kv', 1, 1)),
    'p4': (('wo', 1),),
    4: (('kv', 1, 2), ('kv', 1, 3)),
}
_LOW = 1


def _stage_order(nb):
    ops = []
    for t in range(nb + 2):
        if t < nb:
            ops.append(('qk', t))
        if 2 <= t < nb:
            ops.append(('o', t - 2))
        if 1 <= t <= nb:
            ops.append(('pv', t - 1))
        if t >= nb:
            ops.append(('o', t - 2))
    return ops


def _zero_from(tok):
    t = pltpu.bitcast(tok, jnp.uint32)
    t = lax.shift_right_logical(lax.shift_right_logical(t, jnp.uint32(31)), jnp.uint32(1))
    return pltpu.bitcast(t, jnp.float32)


def _kernel(xa_hbm, ka_hbm, va_hbm, wqa_hbm, woa_hbm,
            xb_hbm, kb_hbm, vb_hbm, wqb_hbm, wob_hbm,
            o_hbm, acc_ref, x_buf, kv_buf, w_buf, o_buf, x_sem, kv_sem, w_sem, o_sem,
            *, rep, sq, d, n_h, nb, ng):
    n_steps = n_h * 2 * ng
    last = n_steps - 1
    hb = n_h.bit_length() - 1

    def coords(st):
        return st >> (hb + 1), (st >> hb) & 1, st & (n_h - 1), st & 1

    scale = _DH ** -0.5 * math.log2(math.e)
    f32, bf16 = jnp.float32, jnp.bfloat16
    mr = rep * sq
    gw = rep * _DH
    n_t = nb * sq // _LANE
    n_grp = len(_GROUPS)
    c_mid = (d // _LANE) * _LANE
    whole = ((0, 0, nb), (1, 0, nb))

    x_hbm = (xa_hbm, xb_hbm)
    kv_hbm = ((ka_hbm, va_hbm), (kb_hbm, vb_hbm))
    w_hbm = ((wqa_hbm, woa_hbm), (wqb_hbm, wob_hbm))

    def x_copy(cs, gg):
        return pltpu.make_async_copy(
            x_hbm[cs].at[pl.ds(gg * nb, nb)], x_buf.at[gg], x_sem.at[gg])

    def w_copy(cs, j, hh, sl, fine):
        col = hh * gw if isinstance(hh, int) else pl.multiple_of(hh * gw, gw)
        sem = w_sem.at[sl * 2 + j] if fine else kv_sem.at[sl * n_grp]
        return pltpu.make_async_copy(
            w_hbm[cs][j].at[:, pl.ds(col, gw)], w_buf.at[sl, j], sem)

    def kv_copy(cs, gg, hh, sl, piece, gi):
        j, i0, i1 = piece
        return pltpu.make_async_copy(
            kv_hbm[cs][j].at[pl.ds(gg * nb + i0, i1 - i0), hh],
            kv_buf.at[sl, j, pl.ds(i0, i1 - i0)],
            kv_sem.at[sl * n_grp + gi])

    def o_copy(gg, t0, t1, c0, c1, si):
        r0 = gg * (nb * sq) + t0 * _LANE
        n_r = (t1 - t0) * _LANE
        return pltpu.make_async_copy(
            o_buf.at[gg, pl.ds(t0 * _LANE, n_r), pl.ds(c0, c1 - c0)],
            o_hbm.at[pl.ds(r0, n_r), pl.ds(c0, c1 - c0)], o_sem.at[si])

    def softmax(s, toks):
        ps, ls = [], []
        sk = s.shape[1]
        for j, r0 in enumerate(range(0, mr, _RC)):
            sc = s[r0:r0 + _RC]
            pm = sc[:, 0:_LANE]
            for cc in range(_LANE, sk, _LANE):
                pm = jnp.maximum(pm, sc[:, cc:cc + _LANE])
            z = _zero_from(toks[j])
            pm = pm + jnp.concatenate([z] * (_RC // 8), axis=0)
            m = jnp.max(pm, axis=-1, keepdims=True)
            e = jnp.exp2(sc - m)
            psum = e[:, 0:_LANE]
            for cc in range(_LANE, sk, _LANE):
                psum = psum + e[:, cc:cc + _LANE]
            ls.append(psum)
            ps.append(e.astype(bf16))
        return jnp.concatenate(ps, axis=0), jnp.concatenate(ls, axis=0)

    def toks_from(y, rounds, n):
        rows, cols = y.shape
        nrb = rows // 16
        cw = cols // rounds
        out = []
        for j in range(n):
            sl = (j * rounds * nrb) // n
            rd, rb = sl // nrb, sl % nrb
            out.append(y[rb * 16:rb * 16 + 8, rd * cw:rd * cw + _LANE])
        return out

    def body(step, special):
        c, g, h, slot = coords(step)
        s, oc, ys = {}, {}, {}
        n_tok = mr // _RC

        def issue(k):
            if k not in _ISSUE:
                return

            @pl.when(step == 0)
            def _():
                for pc in _ISSUE[k]:
                    cc, gg, hh, sl = coords(pc[1])
                    if pc[0] == 'kv':
                        for piece in _GROUPS[pc[2]]:
                            kv_copy(cc, gg, hh, sl, piece, pc[2]).start(priority=_LOW)
                    elif pc[0] == 'x':
                        x_copy(cc, gg).start()
                    else:
                        w_copy(cc, 0 if pc[0] == 'wq' else 1, hh, sl, True).start()

        def prefetch(which):
            if special:
                nc, ngi, nh, nsl = coords(_NFINE)

                @pl.when(step == _NFINE - 1)
                def _():
                    for j in range(2):
                        w_copy(nc, j, nh, nsl, False).start(priority=_LOW)
                    for piece in whole:
                        kv_copy(nc, ngi, nh, nsl, piece, 0).start(priority=_LOW)
                return
            nc, ngi, nh, nsl = coords(step + 1)
            for cs in range(2):
                ok = nc == cs
                if which == 'kv':
                    for piece in whole:
                        @pl.when(ok)
                        def _():
                            kv_copy(cs, ngi, nh, nsl, piece, 0).start()
                else:
                    @pl.when(jnp.logical_and(ok, nh == 0))
                    def _():
                        x_copy(cs, ngi).start()
                    for j in range(2):
                        @pl.when(ok)
                        def _():
                            w_copy(cs, j, nh, nsl, False).start()

        def wait_all():
            for j in range(2):
                w_copy(0, j, h, slot, False).wait()
            for piece in whole:
                kv_copy(0, g, h, slot, piece, 0).wait()

        def out_start(gg, t0, t1, c0, c1, si):
            @pl.when(step == last)
            def _():
                o_copy(gg, t0, t1, c0, c1, si).start()

        if special:
            issue(-1)

            @pl.when(step == 0)
            def _():
                x_copy(0, 0).wait()

            @pl.when(step < _NFINE)
            def _():
                w_copy(0, 0, h, slot, True).wait()
            issue(0)
            prefetch('all')

            @pl.when(step >= _NFINE)
            def _():
                wait_all()
        else:
            @pl.when(h == 0)
            def _():
                x_copy(0, g).wait()
            wait_all()
            prefetch('kv')
        xx = x_buf[g].reshape(nb * sq, d)
        q = jnp.dot(xx[:, c_mid:], w_buf[slot, 0, c_mid:, :], preferred_element_type=f32)
        q = jnp.dot(xx[:, :c_mid], w_buf[slot, 0, :c_mid, :], preferred_element_type=f32) + q
        q = (q * scale).astype(bf16)
        if not special:
            prefetch('w')

        if special:
            for gg, c1, si in ((0, 2 * d, 0), (1, c_mid, 1)):
                for t in range(n_t):
                    yt = acc_ref[gg, t].reshape(2 * d, _LANE)[0:c1]
                    o_buf[gg, t * _LANE:(t + 1) * _LANE, 0:c1] = yt.T.astype(o_buf.dtype)
                out_start(gg, 0, n_t, 0, c1, si)

        def do_qk(n):
            qn = q[n * sq:(n + 1) * sq]
            q2 = jnp.concatenate(
                [qn[:, r * _DH:(r + 1) * _DH] for r in range(rep)], axis=0)
            s[n] = lax.dot_general(q2, kv_buf[slot, 0, n], _NT, preferred_element_type=f32)

        def do_pv(n):
            if n + 1 < nb:
                toks = toks_from(s[n + 1], 4, n_tok)
            else:
                toks = toks_from(ys[n - 2], 1, n_tok)
            p, psum = softmax(s[n], toks)
            o32 = jnp.dot(p, kv_buf[slot, 1, n], preferred_element_type=f32)
            l = jnp.sum(psum + _zero_from(o32[:, 0:_LANE]), axis=-1, keepdims=True)
            r0 = pl.reciprocal(l, approx=True)
            o = o32 * (r0 * (2.0 - l * r0))
            oc[n] = jnp.concatenate([o[r * sq:(r + 1) * sq] for r in range(rep)], axis=1)

        def do_o(n):
            wo = w_buf[slot, 1]
            for t in range((n * sq) // _LANE, ((n + 1) * sq) // _LANE):
                r0, r1 = t * _LANE, (t + 1) * _LANE
                parts = []
                for ii in range(r0 // sq, (r1 - 1) // sq + 1):
                    a, b = max(r0, ii * sq) - ii * sq, min(r1, (ii + 1) * sq) - ii * sq
                    parts.append(oc[ii][a:b])
                ot = jnp.concatenate(parts, axis=0) if len(parts) > 1 else parts[0]
                if special:
                    a_tail = acc_ref[1, t, 0, c_mid:d, :]
                y = lax.dot_general(wo, ot.astype(bf16), _NT, preferred_element_type=f32)
                ys[n] = y
                new = jnp.where(h == 0, 0.0, acc_ref[g, t, c]) + y
                acc_ref[g, t, c] = new
                if special:
                    yt = jnp.concatenate([a_tail, new], axis=0)
                    o_buf[1, r0:r1, c_mid:2 * d] = yt.T.astype(o_buf.dtype)
                    out_start(1, t, t + 1, c_mid, 2 * d, 2)

        for stage in _stage_order(nb):
            if special and stage in _BARS:
                k = _BARS.index(stage)
                issue('p%d' % (k + 1))

                @pl.when(step < _NFINE)
                def _():
                    for piece in _GROUPS[k]:
                        kv_copy(0, g, h, slot, piece, k).wait()
                    if k == _WO_BAR:
                        w_copy(0, 1, h, slot, True).wait()
                issue(k + 1)
            {'qk': do_qk, 'pv': do_pv, 'o': do_o}[stage[0]](stage[1])

        if special:
            @pl.when(step == last)
            def _():
                o_copy(0, 0, n_t, 0, 2 * d, 0).wait()
                o_copy(1, 0, n_t, 0, c_mid, 1).wait()
                for t in range(n_t):
                    o_copy(1, t, t + 1, c_mid, 2 * d, 2).wait()

    i = pl.program_id(0)
    body(jnp.where(i < _NFINE, i, last), True)

    def loop_body(st, carry):
        body(st, False)
        return carry

    lax.fori_loop(_NFINE, jnp.where(i == _NFINE - 1, last, _NFINE), loop_body, 0)


@jax.jit
def pallas_concat_heads__gqa_block_cached__gqa_block_cached__near_ridge_kernel(
    A_x: jax.Array,
    A_k_cache: jax.Array,
    A_v_cache: jax.Array,
    A_wq: jax.Array,
    A_wo: jax.Array,
    B_x: jax.Array,
    B_k_cache: jax.Array,
    B_v_cache: jax.Array,
    B_wq: jax.Array,
    B_wo: jax.Array,
):
    bsz, sq, d = A_x.shape
    _, hkv, sk, dh = A_k_cache.shape
    rep = _HQ // hkv
    gw = rep * dh
    nb = _NB
    ng = bsz // nb
    dt = A_x.dtype
    rows = nb * sq
    assert dh == _DH and ng == 2 and rows % _LANE == 0 and sq % 16 == 0
    assert hkv & (hkv - 1) == 0 and hkv > _NFINE

    any_spec = pl.BlockSpec(memory_space=pl.ANY)
    out = pl.pallas_call(
        functools.partial(_kernel, rep=rep, sq=sq, d=d, n_h=hkv, nb=nb, ng=ng),
        grid=(_NFINE + 1,),
        in_specs=[any_spec] * 10,
        out_specs=any_spec,
        out_shape=jax.ShapeDtypeStruct((bsz * sq, 2 * d), dt),
        scratch_shapes=[pltpu.VMEM((ng, rows // _LANE, 2, d, _LANE), jnp.float32),
                        pltpu.VMEM((ng, nb, sq, d), dt),
                        pltpu.VMEM((2, 2, nb, sk, dh), dt),
                        pltpu.VMEM((2, 2, d, gw), dt),
                        pltpu.VMEM((ng, rows, 2 * d), dt),
                        pltpu.SemaphoreType.DMA((ng,)),
                        pltpu.SemaphoreType.DMA((2 * len(_GROUPS),)),
                        pltpu.SemaphoreType.DMA((4,)),
                        pltpu.SemaphoreType.DMA((3,))],
        compiler_params=pltpu.CompilerParams(
            dimension_semantics=("arbitrary",),
            disable_bounds_checks=True,
            vmem_limit_bytes=100 * 1024 * 1024),
    )(A_x, A_k_cache, A_v_cache, A_wq, A_wo.T, B_x, B_k_cache, B_v_cache, B_wq, B_wo.T)
    return out.reshape(bsz, sq, 2 * d)
```

```python
import functools

import jax
import jax.numpy as jnp
from jax import lax
import jax.experimental.pallas as pl
import jax.experimental.pallas.tpu as pltpu

_HQ = 16
_DH = 256
_NB = 8
_NFINE = 2
_NT = (((1,), (1,)), ((), ()))
_RC = 16
_LANE = 128

_GROUPS = (((0, 0, 2), (1, 0, 1)), ((0, 2, 4), (1, 1, 3)),
           ((0, 4, 6), (1, 3, 5)), ((0, 6, 8), (1, 5, 8)))
_BARS = (('qk', 0), ('qk', 2), ('qk', 4), ('qk', 6))
_WO_BAR = 1
_ISSUE = {
    -1: (('x', 0), ('wq', 0), ('kv', 0, 0), ('kv', 0, 1)),
    0: (('wo', 0),),
    1: (('kv', 0, 2),),
    2: (('kv', 0, 3),),
    'p3': (('wq', 1),),
    3: (('kv', 1, 0), ('kv', 1, 1)),
    'p4': (('wo', 1),),
    4: (('kv', 1, 2), ('kv', 1, 3)),
}
_LOW = 1


def _stage_order(nb):
    ops = []
    for t in range(nb + 2):
        if t < nb:
            ops.append(('qk', t))
        if 2 <= t < nb:
            ops.append(('o', t - 2))
        if 1 <= t <= nb:
            ops.append(('pv', t - 1))
        if t >= nb:
            ops.append(('o', t - 2))
    return ops


def _zero_from(tok):
    t = pltpu.bitcast(tok, jnp.uint32)
    t = lax.shift_right_logical(lax.shift_right_logical(t, jnp.uint32(31)), jnp.uint32(1))
    return pltpu.bitcast(t, jnp.float32)


def _kernel(xa_hbm, ka_hbm, va_hbm, wqa_hbm, woa_hbm,
            xb_hbm, kb_hbm, vb_hbm, wqb_hbm, wob_hbm,
            o_hbm, acc_ref, x_buf, kv_buf, w_buf, o_buf, x_sem, kv_sem, w_sem, o_sem,
            *, rep, sq, d, n_h, nb, ng):
    n_steps = n_h * 2 * ng
    last = n_steps - 1
    hb = n_h.bit_length() - 1

    def coords(st):
        return st >> (hb + 1), (st >> hb) & 1, st & (n_h - 1), st & 1

    scale = _DH ** -0.5
    f32, bf16 = jnp.float32, jnp.bfloat16
    mr = rep * sq
    gw = rep * _DH
    n_t = nb * sq // _LANE
    n_grp = len(_GROUPS)
    c_mid = (d // _LANE) * _LANE
    whole = ((0, 0, nb), (1, 0, nb))

    x_hbm = (xa_hbm, xb_hbm)
    kv_hbm = ((ka_hbm, va_hbm), (kb_hbm, vb_hbm))
    w_hbm = ((wqa_hbm, woa_hbm), (wqb_hbm, wob_hbm))

    def x_copy(cs, gg):
        return pltpu.make_async_copy(
            x_hbm[cs].at[pl.ds(gg * nb, nb)], x_buf.at[gg], x_sem.at[gg])

    def w_copy(cs, j, hh, sl, fine):
        col = hh * gw if isinstance(hh, int) else pl.multiple_of(hh * gw, gw)
        sem = w_sem.at[sl * 2 + j] if fine else kv_sem.at[sl * n_grp]
        return pltpu.make_async_copy(
            w_hbm[cs][j].at[:, pl.ds(col, gw)], w_buf.at[sl, j], sem)

    def kv_copy(cs, gg, hh, sl, piece, gi):
        j, i0, i1 = piece
        return pltpu.make_async_copy(
            kv_hbm[cs][j].at[pl.ds(gg * nb + i0, i1 - i0), hh],
            kv_buf.at[sl, j, pl.ds(i0, i1 - i0)],
            kv_sem.at[sl * n_grp + gi])

    def o_copy(gg, t0, t1, c0, c1, si):
        r0 = gg * (nb * sq) + t0 * _LANE
        n_r = (t1 - t0) * _LANE
        return pltpu.make_async_copy(
            o_buf.at[gg, pl.ds(t0 * _LANE, n_r), pl.ds(c0, c1 - c0)],
            o_hbm.at[pl.ds(r0, n_r), pl.ds(c0, c1 - c0)], o_sem.at[si])

    def softmax(s, toks, late):
        ps, ls = [], []
        sk = s.shape[1]
        for j, r0 in enumerate(range(0, mr, _RC)):
            sc = s[r0:r0 + _RC]
            pm = sc[:, 0:_LANE]
            for cc in range(_LANE, sk, _LANE):
                pm = jnp.maximum(pm, sc[:, cc:cc + _LANE])
            z = _zero_from(toks[j])
            pm = pm + jnp.concatenate([z] * (_RC // 8), axis=0)
            m = jnp.max(pm, axis=-1, keepdims=True)
            e = jnp.exp(sc - m)
            psum = e[:, 0:_LANE]
            for cc in range(_LANE, sk, _LANE):
                psum = psum + e[:, cc:cc + _LANE]
            ls.append(psum)
            ps.append(e if late else e.astype(bf16))
        return jnp.concatenate(ps, axis=0).astype(bf16), jnp.concatenate(ls, axis=0)

    def toks_from(y, rounds, n):
        rows, cols = y.shape
        nrb = rows // 16
        cw = cols // rounds
        out = []
        for j in range(n):
            sl = (j * rounds * nrb) // n
            rd, rb = sl // nrb, sl % nrb
            out.append(y[rb * 16:rb * 16 + 8, rd * cw:rd * cw + _LANE])
        return out

    def body(step, special):
        c, g, h, slot = coords(step)
        s, oc, ys = {}, {}, {}
        n_tok = mr // _RC
        late = special

        def issue(k):
            if k not in _ISSUE:
                return

            @pl.when(step == 0)
            def _():
                for pc in _ISSUE[k]:
                    cc, gg, hh, sl = coords(pc[1])
                    if pc[0] == 'kv':
                        for piece in _GROUPS[pc[2]]:
                            kv_copy(cc, gg, hh, sl, piece, pc[2]).start(priority=_LOW)
                    elif pc[0] == 'x':
                        x_copy(cc, gg).start()
                    else:
                        w_copy(cc, 0 if pc[0] == 'wq' else 1, hh, sl, True).start()

        def prefetch(which):
            if special:
                nc, ngi, nh, nsl = coords(_NFINE)

                @pl.when(step == _NFINE - 1)
                def _():
                    for j in range(2):
                        w_copy(nc, j, nh, nsl, False).start(priority=_LOW)
                    for piece in whole:
                        kv_copy(nc, ngi, nh, nsl, piece, 0).start(priority=_LOW)
                return
            nc, ngi, nh, nsl = coords(step + 1)
            for cs in range(2):
                ok = nc == cs
                if which == 'kv':
                    for piece in whole:
                        @pl.when(ok)
                        def _():
                            kv_copy(cs, ngi, nh, nsl, piece, 0).start()
                else:
                    @pl.when(jnp.logical_and(ok, nh == 0))
                    def _():
                        x_copy(cs, ngi).start()
                    for j in range(2):
                        @pl.when(ok)
                        def _():
                            w_copy(cs, j, nh, nsl, False).start()

        def wait_all():
            for j in range(2):
                w_copy(0, j, h, slot, False).wait()
            for piece in whole:
                kv_copy(0, g, h, slot, piece, 0).wait()

        def out_start(gg, t0, t1, c0, c1, si):
            @pl.when(step == last)
            def _():
                o_copy(gg, t0, t1, c0, c1, si).start()

        if special:
            issue(-1)

            @pl.when(step == 0)
            def _():
                x_copy(0, 0).wait()

            @pl.when(step < _NFINE)
            def _():
                w_copy(0, 0, h, slot, True).wait()
            issue(0)
            prefetch('all')

            @pl.when(step >= _NFINE)
            def _():
                wait_all()
        else:
            @pl.when(h == 0)
            def _():
                x_copy(0, g).wait()
            wait_all()
            prefetch('kv')
        xx = x_buf[g].reshape(nb * sq, d)
        q = jnp.dot(xx[:, c_mid:], w_buf[slot, 0, c_mid:, :], preferred_element_type=f32)
        q = jnp.dot(xx[:, :c_mid], w_buf[slot, 0, :c_mid, :], preferred_element_type=f32) + q
        q = q * scale if late else (q * scale).astype(bf16)
        if not special:
            prefetch('w')

        if special:
            for gg, c1, si in ((0, 2 * d, 0), (1, c_mid, 1)):
                for t in range(n_t):
                    yt = acc_ref[gg, t].reshape(2 * d, _LANE)[0:c1]
                    o_buf[gg, t * _LANE:(t + 1) * _LANE, 0:c1] = yt.T.astype(o_buf.dtype)
                out_start(gg, 0, n_t, 0, c1, si)

        def do_qk(n):
            qn = q[n * sq:(n + 1) * sq]
            q2 = jnp.concatenate(
                [qn[:, r * _DH:(r + 1) * _DH] for r in range(rep)], axis=0).astype(bf16)
            s[n] = lax.dot_general(q2, kv_buf[slot, 0, n], _NT, preferred_element_type=f32)

        def do_pv(n):
            if n + 1 < nb:
                toks = toks_from(s[n + 1], 4, n_tok)
            else:
                toks = toks_from(ys[n - 2], 1, n_tok)
            p, psum = softmax(s[n], toks, late)
            o32 = jnp.dot(p, kv_buf[slot, 1, n], preferred_element_type=f32)
            l = jnp.sum(psum + _zero_from(o32[:, 0:_LANE]), axis=-1, keepdims=True)
            r0 = pl.reciprocal(l, approx=True)
            o = o32 * (r0 * (2.0 - l * r0))
            if not late:
                o = o.astype(bf16)
            oc[n] = jnp.concatenate([o[r * sq:(r + 1) * sq] for r in range(rep)], axis=1)

        def do_o(n):
            wo = w_buf[slot, 1]
            for t in range((n * sq) // _LANE, ((n + 1) * sq) // _LANE):
                r0, r1 = t * _LANE, (t + 1) * _LANE
                parts = []
                for ii in range(r0 // sq, (r1 - 1) // sq + 1):
                    a, b = max(r0, ii * sq) - ii * sq, min(r1, (ii + 1) * sq) - ii * sq
                    parts.append(oc[ii][a:b])
                ot = jnp.concatenate(parts, axis=0) if len(parts) > 1 else parts[0]
                if special:
                    a_tail = acc_ref[1, t, 0, c_mid:d, :]
                y = lax.dot_general(wo, ot.astype(bf16), _NT, preferred_element_type=f32)
                ys[n] = y
                new = jnp.where(h == 0, 0.0, acc_ref[g, t, c]) + y
                acc_ref[g, t, c] = new
                if special:
                    yt = jnp.concatenate([a_tail, new], axis=0)
                    o_buf[1, r0:r1, c_mid:2 * d] = yt.T.astype(o_buf.dtype)
                    out_start(1, t, t + 1, c_mid, 2 * d, 2)

        for stage in _stage_order(nb):
            if special and stage in _BARS:
                k = _BARS.index(stage)
                issue('p%d' % (k + 1))

                @pl.when(step < _NFINE)
                def _():
                    for piece in _GROUPS[k]:
                        kv_copy(0, g, h, slot, piece, k).wait()
                    if k == _WO_BAR:
                        w_copy(0, 1, h, slot, True).wait()
                issue(k + 1)
            {'qk': do_qk, 'pv': do_pv, 'o': do_o}[stage[0]](stage[1])

        if special:
            @pl.when(step == last)
            def _():
                o_copy(0, 0, n_t, 0, 2 * d, 0).wait()
                o_copy(1, 0, n_t, 0, c_mid, 1).wait()
                for t in range(n_t):
                    o_copy(1, t, t + 1, c_mid, 2 * d, 2).wait()

    i = pl.program_id(0)
    body(jnp.where(i < _NFINE, i, last), True)

    def loop_body(st, carry):
        body(st, False)
        return carry

    lax.fori_loop(_NFINE, jnp.where(i == _NFINE - 1, last, _NFINE), loop_body, 0)


@jax.jit
def pallas_concat_heads__gqa_block_cached__gqa_block_cached__near_ridge_kernel(
    A_x: jax.Array,
    A_k_cache: jax.Array,
    A_v_cache: jax.Array,
    A_wq: jax.Array,
    A_wo: jax.Array,
    B_x: jax.Array,
    B_k_cache: jax.Array,
    B_v_cache: jax.Array,
    B_wq: jax.Array,
    B_wo: jax.Array,
):
    bsz, sq, d = A_x.shape
    _, hkv, sk, dh = A_k_cache.shape
    rep = _HQ // hkv
    gw = rep * dh
    nb = _NB
    ng = bsz // nb
    dt = A_x.dtype
    rows = nb * sq
    assert dh == _DH and ng == 2 and rows % _LANE == 0 and sq % 16 == 0
    assert hkv & (hkv - 1) == 0 and hkv > _NFINE

    any_spec = pl.BlockSpec(memory_space=pl.ANY)
    out = pl.pallas_call(
        functools.partial(_kernel, rep=rep, sq=sq, d=d, n_h=hkv, nb=nb, ng=ng),
        grid=(_NFINE + 1,),
        in_specs=[any_spec] * 10,
        out_specs=any_spec,
        out_shape=jax.ShapeDtypeStruct((bsz * sq, 2 * d), dt),
        scratch_shapes=[pltpu.VMEM((ng, rows // _LANE, 2, d, _LANE), jnp.float32),
                        pltpu.VMEM((ng, nb, sq, d), dt),
                        pltpu.VMEM((2, 2, nb, sk, dh), dt),
                        pltpu.VMEM((2, 2, d, gw), dt),
                        pltpu.VMEM((ng, rows, 2 * d), dt),
                        pltpu.SemaphoreType.DMA((ng,)),
                        pltpu.SemaphoreType.DMA((2 * len(_GROUPS),)),
                        pltpu.SemaphoreType.DMA((4,)),
                        pltpu.SemaphoreType.DMA((3,))],
        compiler_params=pltpu.CompilerParams(
            dimension_semantics=("arbitrary",),
            disable_bounds_checks=True,
            vmem_limit_bytes=100 * 1024 * 1024),
    )(A_x, A_k_cache, A_v_cache, A_wq, A_wo.T, B_x, B_k_cache, B_v_cache, B_wq, B_wo.T)
    return out.reshape(bsz, sq, 2 * d)
```

```python
import functools

import jax
import jax.numpy as jnp
from jax import lax
import jax.experimental.pallas as pl
import jax.experimental.pallas.tpu as pltpu

_HQ = 16
_DH = 256
_NB = 8
_NFINE = 2
_NT = (((1,), (1,)), ((), ()))
_RC = 16
_LANE = 128

_GROUPS = (((0, 0, 2), (1, 0, 1)), ((0, 2, 4), (1, 1, 3)),
           ((0, 4, 6), (1, 3, 5)), ((0, 6, 8), (1, 5, 8)))
_BARS = (('qk', 0), ('qk', 2), ('qk', 4), ('qk', 6))
_WO_BAR = 1
_ISSUE = {
    -1: (('x', 0), ('wq', 0), ('kv', 0, 0), ('kv', 0, 1)),
    0: (('wo', 0),),
    1: (('kv', 0, 2),),
    2: (('kv', 0, 3),),
    'p3': (('wq', 1),),
    3: (('kv', 1, 0), ('kv', 1, 1)),
    'p4': (('wo', 1),),
    4: (('kv', 1, 2), ('kv', 1, 3)),
}
_LOW = 1


def _stage_order(nb):
    ops = []
    for t in range(nb + 2):
        if t < nb:
            ops.append(('qk', t))
        if 2 <= t < nb:
            ops.append(('o', t - 2))
        if 1 <= t <= nb:
            ops.append(('pv', t - 1))
        if t >= nb:
            ops.append(('o', t - 2))
    return ops


def _zero_from(tok):
    t = pltpu.bitcast(tok, jnp.uint32)
    t = lax.shift_right_logical(lax.shift_right_logical(t, jnp.uint32(31)), jnp.uint32(1))
    return pltpu.bitcast(t, jnp.float32)


def _kernel(xa_hbm, ka_hbm, va_hbm, wqa_hbm, woa_hbm,
            xb_hbm, kb_hbm, vb_hbm, wqb_hbm, wob_hbm,
            o_hbm, acc_ref, x_buf, kv_buf, w_buf, o_buf, x_sem, kv_sem, w_sem, o_sem,
            *, rep, sq, d, n_h, nb, ng):
    n_steps = n_h * 2 * ng
    last = n_steps - 1
    hb = n_h.bit_length() - 1

    def coords(st):
        return st >> (hb + 1), (st >> hb) & 1, st & (n_h - 1), st & 1

    scale = _DH ** -0.5
    f32, bf16 = jnp.float32, jnp.bfloat16
    mr = rep * sq
    gw = rep * _DH
    n_t = nb * sq // _LANE
    n_grp = len(_GROUPS)
    c_mid = (d // _LANE) * _LANE
    whole = ((0, 0, nb), (1, 0, nb))

    x_hbm = (xa_hbm, xb_hbm)
    kv_hbm = ((ka_hbm, va_hbm), (kb_hbm, vb_hbm))
    w_hbm = ((wqa_hbm, woa_hbm), (wqb_hbm, wob_hbm))

    def x_copy(cs, gg):
        return pltpu.make_async_copy(
            x_hbm[cs].at[pl.ds(gg * nb, nb)], x_buf.at[gg], x_sem.at[gg])

    def w_copy(cs, j, hh, sl, fine):
        col = hh * gw if isinstance(hh, int) else pl.multiple_of(hh * gw, gw)
        sem = w_sem.at[sl * 2 + j] if fine else kv_sem.at[sl * n_grp]
        return pltpu.make_async_copy(
            w_hbm[cs][j].at[:, pl.ds(col, gw)], w_buf.at[sl, j], sem)

    def kv_copy(cs, gg, hh, sl, piece, gi):
        j, i0, i1 = piece
        return pltpu.make_async_copy(
            kv_hbm[cs][j].at[pl.ds(gg * nb + i0, i1 - i0), hh],
            kv_buf.at[sl, j, pl.ds(i0, i1 - i0)],
            kv_sem.at[sl * n_grp + gi])

    def o_copy(gg, t0, t1, c0, c1, si):
        r0 = gg * (nb * sq) + t0 * _LANE
        n_r = (t1 - t0) * _LANE
        return pltpu.make_async_copy(
            o_buf.at[gg, pl.ds(t0 * _LANE, n_r), pl.ds(c0, c1 - c0)],
            o_hbm.at[pl.ds(r0, n_r), pl.ds(c0, c1 - c0)], o_sem.at[si])

    def softmax(s, toks, late):
        ps, ls = [], []
        sk = s.shape[1]
        for j, r0 in enumerate(range(0, mr, _RC)):
            sc = s[r0:r0 + _RC]
            pm = sc[:, 0:_LANE]
            for cc in range(_LANE, sk, _LANE):
                pm = jnp.maximum(pm, sc[:, cc:cc + _LANE])
            z = _zero_from(toks[j])
            pm = pm + jnp.concatenate([z] * (_RC // 8), axis=0)
            m = jnp.max(pm, axis=-1, keepdims=True)
            e = jnp.exp(sc - m)
            psum = e[:, 0:_LANE]
            for cc in range(_LANE, sk, _LANE):
                psum = psum + e[:, cc:cc + _LANE]
            ls.append(psum)
            ps.append(e if late else e.astype(bf16))
        return jnp.concatenate(ps, axis=0).astype(bf16), jnp.concatenate(ls, axis=0)

    def toks_from(y, rounds, n):
        rows, cols = y.shape
        nrb = rows // 16
        cw = cols // rounds
        out = []
        for j in range(n):
            sl = (j * rounds * nrb) // n
            rd, rb = sl // nrb, sl % nrb
            out.append(y[rb * 16:rb * 16 + 8, rd * cw:rd * cw + _LANE])
        return out

    def body(step, special):
        c, g, h, slot = coords(step)
        s, oc, ys = {}, {}, {}
        n_tok = mr // _RC
        late = special

        def issue(k):
            if k not in _ISSUE:
                return

            @pl.when(step == 0)
            def _():
                for pc in _ISSUE[k]:
                    cc, gg, hh, sl = coords(pc[1])
                    if pc[0] == 'kv':
                        for piece in _GROUPS[pc[2]]:
                            kv_copy(cc, gg, hh, sl, piece, pc[2]).start(priority=_LOW)
                    elif pc[0] == 'x':
                        x_copy(cc, gg).start()
                    else:
                        w_copy(cc, 0 if pc[0] == 'wq' else 1, hh, sl, True).start()

        def prefetch(which):
            if special:
                nc, ngi, nh, nsl = coords(_NFINE)

                @pl.when(step == _NFINE - 1)
                def _():
                    for j in range(2):
                        w_copy(nc, j, nh, nsl, False).start(priority=_LOW)
                    for piece in whole:
                        kv_copy(nc, ngi, nh, nsl, piece, 0).start(priority=_LOW)
                return
            nc, ngi, nh, nsl = coords(step + 1)
            for cs in range(2):
                ok = nc == cs
                if which == 'kv':
                    for piece in whole:
                        @pl.when(ok)
                        def _():
                            kv_copy(cs, ngi, nh, nsl, piece, 0).start()
                else:
                    @pl.when(jnp.logical_and(ok, nh == 0))
                    def _():
                        x_copy(cs, ngi).start()
                    for j in range(2):
                        @pl.when(ok)
                        def _():
                            w_copy(cs, j, nh, nsl, False).start()

        def wait_all():
            for j in range(2):
                w_copy(0, j, h, slot, False).wait()
            for piece in whole:
                kv_copy(0, g, h, slot, piece, 0).wait()

        def out_start(gg, t0, t1, c0, c1, si):
            @pl.when(step == last)
            def _():
                o_copy(gg, t0, t1, c0, c1, si).start()

        if special:
            issue(-1)

            @pl.when(step == 0)
            def _():
                x_copy(0, 0).wait()

            @pl.when(step < _NFINE)
            def _():
                w_copy(0, 0, h, slot, True).wait()
            issue(0)
            prefetch('all')

            @pl.when(step >= _NFINE)
            def _():
                wait_all()
        else:
            @pl.when(h == 0)
            def _():
                x_copy(0, g).wait()
            wait_all()
            prefetch('kv')
        xx = x_buf[g].reshape(nb * sq, d)
        q = jnp.dot(xx[:, c_mid:], w_buf[slot, 0, c_mid:, :], preferred_element_type=f32)
        q = jnp.dot(xx[:, :c_mid], w_buf[slot, 0, :c_mid, :], preferred_element_type=f32) + q
        q = q * scale if late else (q * scale).astype(bf16)
        if not special:
            prefetch('w')

        if special:
            for gg, c1, si in ((0, 2 * d, 0), (1, c_mid, 1)):
                for t in range(n_t):
                    yt = acc_ref[gg, t].reshape(2 * d, _LANE)[0:c1]
                    o_buf[gg, t * _LANE:(t + 1) * _LANE, 0:c1] = yt.T.astype(o_buf.dtype)
                out_start(gg, 0, n_t, 0, c1, si)

        def do_qk(n):
            qn = q[n * sq:(n + 1) * sq]
            q2 = jnp.concatenate(
                [qn[:, r * _DH:(r + 1) * _DH] for r in range(rep)], axis=0).astype(bf16)
            s[n] = lax.dot_general(q2, kv_buf[slot, 0, n], _NT, preferred_element_type=f32)

        def do_pv(n):
            if n + 1 < nb:
                toks = toks_from(s[n + 1], 4, n_tok)
            else:
                toks = toks_from(ys[n - 2], 1, n_tok)
            p, psum = softmax(s[n], toks, late)
            o32 = jnp.dot(p, kv_buf[slot, 1, n], preferred_element_type=f32)
            l = jnp.sum(psum + _zero_from(o32[:, 0:_LANE]), axis=-1, keepdims=True)
            r0 = pl.reciprocal(l, approx=True)
            o = o32 * (r0 * (2.0 - l * r0))
            if not late:
                o = o.astype(bf16)
            oc[n] = jnp.concatenate([o[r * sq:(r + 1) * sq] for r in range(rep)], axis=1)

        def do_o(n):
            wo = w_buf[slot, 1]
            for t in range((n * sq) // _LANE, ((n + 1) * sq) // _LANE):
                r0, r1 = t * _LANE, (t + 1) * _LANE
                parts = []
                for ii in range(r0 // sq, (r1 - 1) // sq + 1):
                    a, b = max(r0, ii * sq) - ii * sq, min(r1, (ii + 1) * sq) - ii * sq
                    parts.append(oc[ii][a:b])
                ot = jnp.concatenate(parts, axis=0) if len(parts) > 1 else parts[0]
                if special:
                    a_tail = acc_ref[1, t, 0, c_mid:d, :]
                y = lax.dot_general(wo, ot.astype(bf16), _NT, preferred_element_type=f32)
                ys[n] = y
                new = jnp.where(h == 0, 0.0, acc_ref[g, t, c]) + y
                acc_ref[g, t, c] = new
                if special:
                    yt = jnp.concatenate([a_tail, new], axis=0)
                    if t < n_t - 1:
                        o_buf[1, r0:r1, c_mid:2 * d] = yt.T.astype(o_buf.dtype)
                        out_start(1, t, t + 1, c_mid, 2 * d, 2)
                    else:
                        @pl.when(step == last)
                        def _():
                            o_buf[1, r0:r1, c_mid:2 * d] = yt.T.astype(o_buf.dtype)
                            o_copy(1, t, t + 1, c_mid, 2 * d, 2).start()

        for stage in _stage_order(nb):
            if special and stage in _BARS:
                k = _BARS.index(stage)
                issue('p%d' % (k + 1))

                @pl.when(step < _NFINE)
                def _():
                    for piece in _GROUPS[k]:
                        kv_copy(0, g, h, slot, piece, k).wait()
                    if k == _WO_BAR:
                        w_copy(0, 1, h, slot, True).wait()
                issue(k + 1)
            {'qk': do_qk, 'pv': do_pv, 'o': do_o}[stage[0]](stage[1])

        if special:
            @pl.when(step == last)
            def _():
                o_copy(0, 0, n_t, 0, 2 * d, 0).wait()
                o_copy(1, 0, n_t, 0, c_mid, 1).wait()
                for t in range(n_t):
                    o_copy(1, t, t + 1, c_mid, 2 * d, 2).wait()

    i = pl.program_id(0)
    body(jnp.where(i < _NFINE, i, last), True)

    def loop_body(st, carry):
        body(st, False)
        return carry

    lax.fori_loop(_NFINE, jnp.where(i == _NFINE - 1, last, _NFINE), loop_body, 0)


@jax.jit
def pallas_concat_heads__gqa_block_cached__gqa_block_cached__near_ridge_kernel(
    A_x: jax.Array,
    A_k_cache: jax.Array,
    A_v_cache: jax.Array,
    A_wq: jax.Array,
    A_wo: jax.Array,
    B_x: jax.Array,
    B_k_cache: jax.Array,
    B_v_cache: jax.Array,
    B_wq: jax.Array,
    B_wo: jax.Array,
):
    bsz, sq, d = A_x.shape
    _, hkv, sk, dh = A_k_cache.shape
    rep = _HQ // hkv
    gw = rep * dh
    nb = _NB
    ng = bsz // nb
    dt = A_x.dtype
    rows = nb * sq
    assert dh == _DH and ng == 2 and rows % _LANE == 0 and sq % 16 == 0
    assert hkv & (hkv - 1) == 0 and hkv > _NFINE

    any_spec = pl.BlockSpec(memory_space=pl.ANY)
    out = pl.pallas_call(
        functools.partial(_kernel, rep=rep, sq=sq, d=d, n_h=hkv, nb=nb, ng=ng),
        grid=(_NFINE + 1,),
        in_specs=[any_spec] * 10,
        out_specs=any_spec,
        out_shape=jax.ShapeDtypeStruct((bsz * sq, 2 * d), dt),
        scratch_shapes=[pltpu.VMEM((ng, rows // _LANE, 2, d, _LANE), jnp.float32),
                        pltpu.VMEM((ng, nb, sq, d), dt),
                        pltpu.VMEM((2, 2, nb, sk, dh), dt),
                        pltpu.VMEM((2, 2, d, gw), dt),
                        pltpu.VMEM((ng, rows, 2 * d), dt),
                        pltpu.SemaphoreType.DMA((ng,)),
                        pltpu.SemaphoreType.DMA((2 * len(_GROUPS),)),
                        pltpu.SemaphoreType.DMA((4,)),
                        pltpu.SemaphoreType.DMA((3,))],
        compiler_params=pltpu.CompilerParams(
            dimension_semantics=("arbitrary",),
            disable_bounds_checks=True,
            vmem_limit_bytes=100 * 1024 * 1024),
    )(A_x, A_k_cache, A_v_cache, A_wq, A_wo.T, B_x, B_k_cache, B_v_cache, B_wq, B_wo.T)
    return out.reshape(bsz, sq, 2 * d)
```
